```python
import jax
import jax.numpy as jnp

def _softmax(x, axis=-1):
    return jax.nn.softmax(x, axis=axis)

def _gelu(x):
    return jax.nn.gelu(x, approximate=True)

def _silu(x):
    return jax.nn.silu(x)

def _sigmoid(x):
    return jax.nn.sigmoid(x)

def _layernorm(x, axis=-1, eps=1e-05):
    m = jnp.mean(x, axis=axis, keepdims=True)
    v = jnp.var(x, axis=axis, keepdims=True)
    return (x - m) / jnp.sqrt(v + eps)

def _scatter_add(tgt, idx, src, axis=0):
    return tgt.at[idx].add(src)

def _segment_sum(src, seg, n):
    return jax.ops.segment_sum(src, seg, n)

class _Rng:

    def __init__(self, key):
        self._k = key

    def _next(self):
        self._k, sub = jax.random.split(self._k)
        return sub

    def normal(self, shape):
        return jax.random.normal(self._next(), shape, dtype=jnp.bfloat16)

    def randint(self, lo, hi, shape):
        return jax.random.randint(self._next(), shape, lo, hi, dtype=jnp.int32)

    def uniform(self, shape, lo=0.0, hi=1.0):
        return jax.random.uniform(self._next(), shape, jnp.bfloat16, lo, hi)

    def permutation(self, n):
        return jax.random.permutation(self._next(), n)
kernel_name = 'adaLN_cond__memory_aug_infini_attn__dense_activation_gelu__prompt'

def _fwd_setup_inputs():
    _rng = _Rng(jax.random.key(int.from_bytes(__import__("os").urandom(4), "little")))
    _w = lambda a: (lambda t: t.astype(jnp.bfloat16) if jnp.issubdtype(t.dtype, jnp.floating) else t)(jnp.asarray(a))

    def _A_setup():
        B, S, D, H = (1, 2048, 640, 32)
        N = 4
        L = max(1, S // N)
        sc = D ** (-0.5)
        return {'x': _w((lambda *s: _rng.normal(s) * 0.05)(B, N * L, D)), 'wq': _w((lambda *s: _rng.normal(s) * 0.05)(D, D) * sc), 'wk': _w((lambda *s: _rng.normal(s) * 0.05)(D, D) * sc), 'wv': _w((lambda *s: _rng.normal(s) * 0.05)(D, D) * sc), 'wo': _w((lambda *s: _rng.normal(s) * 0.05)(D, D) * sc), 'beta': _w((lambda *s: _rng.normal(s) * 0.05)(H))}
    _A_in = _A_setup()

    def _B_setup():
        B, S, D, F = (1, 2048, 640, 1728)
        return {'x': _w((lambda *s: _rng.normal(s) * 0.05)(B, S, D)), 'w1': _w((lambda *s: _rng.normal(s) * 0.05)(D, F) * D ** (-0.5)), 'b1': _w((lambda *s: _rng.normal(s) * 0.05)(F) * 0.01), 'w2': _w((lambda *s: _rng.normal(s) * 0.05)(F, D) * F ** (-0.5)), 'b2': _w((lambda *s: _rng.normal(s) * 0.05)(D) * 0.01)}
    _B_in = _B_setup()
    return {'A_x': _A_in['x'], 'A_wq': _A_in['wq'], 'A_wk': _A_in['wk'], 'A_wv': _A_in['wv'], 'A_wo': _A_in['wo'], 'A_beta': _A_in['beta'], 'B_x': _B_in['x'], 'B_w1': _B_in['w1'], 'B_b1': _B_in['b1'], 'B_w2': _B_in['w2'], 'B_b2': _B_in['b2'], 'c': _w((lambda *s: _rng.normal(s) * 0.05)(1, 640)), 'w_mod': _w((lambda *s: _rng.normal(s) * 0.05)(640, 6 * 640) * 640 ** (-0.5))}

def _fwd_reference(A_x, A_wq, A_wk, A_wv, A_wo, A_beta, B_x, B_w1, B_b1, B_w2, B_b2, c, w_mod):

    def _A_ref(x, wq, wk, wv, wo, beta):
        B, S, D = x.shape
        H = 32
        Dh = D // H
        N = 4
        L = S // N
        q = (lambda x, *d: x.transpose(*d))((x @ wq).reshape(B, S, H, Dh), 0, 2, 1, 3).reshape(B, H, N, L, Dh)
        k = (lambda x, *d: x.transpose(*d))((x @ wk).reshape(B, S, H, Dh), 0, 2, 1, 3).reshape(B, H, N, L, Dh)
        v = (lambda x, *d: x.transpose(*d))((x @ wv).reshape(B, S, H, Dh), 0, 2, 1, 3).reshape(B, H, N, L, Dh)
        phi = lambda t: jnp.where(t > 0, t + 1.0, jnp.exp(t))
        scale = Dh ** (-0.5)
        ar = jnp.arange(L)
        mask = (lambda x, dt: x.astype(dt))(ar[:, None] < ar[None, :], x.dtype) * -1000000000.0
        g = _sigmoid(beta).reshape(1, H, 1, 1)
        M = jnp.einsum('bhd,bhe->bhde', q[:, :, 0, 0, :] * 0.0, q[:, :, 0, 0, :] * 0.0)
        z = q[:, :, 0, 0, :] * 0.0
        outs = []
        for s in range(N):
            qs, ks, vs = (q[:, :, s].copy(), k[:, :, s].copy(), v[:, :, s].copy())
            logits = jnp.einsum('bhqd,bhkd->bhqk', qs, ks) * scale + mask
            p = _softmax(logits, axis=-1)
            a_dot = jnp.einsum('bhqk,bhkd->bhqd', p, vs)
            pq = phi(qs)
            num = jnp.einsum('bhld,bhde->bhle', pq, M)
            den = jnp.einsum('bhld,bhd->bhl', pq, z)[..., None] + 1e-06
            a_mem = num / den
            o = g * a_mem + (1.0 - g) * a_dot
            outs.append(o)
            pk = phi(ks)
            M = M + jnp.einsum('bhld,bhle->bhde', pk, vs)
            z = z + jnp.einsum('bhld->bhd', pk)
        o = (lambda x, *d: x.transpose(*d))(jnp.stack(outs, 2).reshape(B, H, S, Dh), 0, 2, 1, 3).reshape(B, S, D)
        return o @ wo

    def _B_ref(x, w1, b1, w2, b2):
        h = jnp.einsum('bsd,df->bsf', x, w1) + b1
        h = _gelu(h)
        return jnp.einsum('bsf,fd->bsd', h, w2) + b2
    x = A_x
    mod = (_silu(c) @ w_mod).reshape(c.shape[0], 6, 1, -1)
    sa, ca, ga, sb, cb, gb = (mod[:, 0].copy(), mod[:, 1].copy(), mod[:, 2].copy(), mod[:, 3].copy(), mod[:, 4].copy(), mod[:, 5].copy())
    h = _layernorm(x, axis=-1) * (1 + ca) + sa
    x = x + ga * _A_ref(h, A_wq, A_wk, A_wv, A_wo, A_beta)
    h = _layernorm(x, axis=-1) * (1 + cb) + sb
    x = x + gb * _B_ref(h, B_w1, B_b1, B_w2, B_b2)
    return x

def setup_inputs():
    _inp = _fwd_setup_inputs()
    _gk = jax.random.fold_in(jax.random.key(int.from_bytes(__import__("os").urandom(4), "little")), 2 ** 31 - 1)
    _shapes = [[1, 2048, 640]]
    _dtypes = ['bfloat16']
    _gks = jax.random.split(_gk, len(_shapes))
    _gs = [jax.random.normal(k, s, dtype=jnp.dtype(d)) * 0.05 for k, s, d in zip(_gks, _shapes, _dtypes)]
    _inp['grad_out'] = _gs[0]
    return _inp

def reference(A_x, A_wq, A_wk, A_wv, A_wo, A_beta, B_w1, B_b1, B_w2, B_b2, c, w_mod, B_x, grad_out):
    _const = dict(B_x=B_x)

    def _f(*_d):
        return _fwd_reference(**{'A_x': _d[0], 'A_wq': _d[1], 'A_wk': _d[2], 'A_wv': _d[3], 'A_wo': _d[4], 'A_beta': _d[5], 'B_w1': _d[6], 'B_b1': _d[7], 'B_w2': _d[8], 'B_b2': _d[9], 'c': _d[10], 'w_mod': _d[11], **_const})
    _out, _vjp = jax.vjp(_f, A_x, A_wq, A_wk, A_wv, A_wo, A_beta, B_w1, B_b1, B_w2, B_b2, c, w_mod)
    _grads = _vjp(grad_out)
    _out0 = jnp.asarray(_out)
    return (_out0, *[jnp.asarray(_g) for _g in _grads])
```

```python
import math

import jax
import jax.numpy as jnp
from jax import lax
import jax.experimental.pallas as pl
import jax.experimental.pallas.tpu as pltpu

BF = jnp.bfloat16
F32 = jnp.float32

S_LEN = 2048
D = 640
H = 32
DH = 20
NSEG = 4
L = 512
F = 1728
FP = 1792
FR = 576
FQ = 144
NG = 8
EPS = 1e-5
SCALE = DH ** -0.5
LOG2E = math.log2(math.e)
GELU_C = math.sqrt(2.0 / math.pi)
GELU_A = 0.044715

NN = (((1,), (0,)), ((), ()))
NT = (((1,), (1,)), ((), ()))
TN = (((0,), (0,)), ((), ()))

PIECES = [(j, i) for j in range(4) for i in range(j + 1)]
FWD_LAG = 6
BWD_LAG = 2


def _dot(a, b, dims=NN):
    return lax.dot_general(a, b, dims, preferred_element_type=F32)


def _blockdiag(x):
    cols = []
    for hh in range(4):
        parts = []
        if hh > 0:
            parts.append(jnp.zeros((32 * hh, 128), x.dtype))
        parts.append(x[32 * hh:32 * hh + 32])
        if hh < 3:
            parts.append(jnp.zeros((96 - 32 * hh, 128), x.dtype))
        cols.append(jnp.concatenate(parts, axis=0))
    return jnp.concatenate(cols, axis=1)


def _colsum8(v):
    r, c = v.shape
    return jnp.sum(v.reshape(r // 8, 8, c), axis=0)


def _phi(t):
    return jnp.where(t > 0, t + 1.0, jnp.exp(jnp.minimum(t, 0.0)))


def _ln_stats(x):
    mu = jnp.mean(x, axis=-1, keepdims=True)
    xc = x - mu
    var = jnp.mean(xc * xc, axis=-1, keepdims=True)
    rstd = lax.rsqrt(var + EPS)
    return xc * rstd, rstd


def _ln_bwd(dxhat, xhat, rstd):
    m1 = jnp.mean(dxhat, axis=-1, keepdims=True)
    m2 = jnp.mean(dxhat * xhat, axis=-1, keepdims=True)
    return rstd * (dxhat - m1 - xhat * m2)


def _kernel(
    x_hbm, wq_hbm, wk_hbm, wv_hbm, wo_hbm, beta_ref, w1_hbm, b1_ref, w2_hbm, b2_ref,
    c_ref, wmod_hbm, go_hbm,
    out_hbm, dx_hbm, dwq_hbm, dwk_hbm, dwv_hbm, dwo_hbm, dbeta_ref, dw1_hbm, db1_ref,
    dw2_hbm, db2_ref, dc_ref, dwmod_hbm,
    wmod_v, wraw_v, wqkvT_v, wo_v, w1_v, w2_v, x_v, go_v,
    mod_v, b1c_v, gT_v, bias_v, scol_v, dsil_v,
    h1T_v, hA_v, QT, KT, VT, KN, VN, MTs, Ms, Macc, T_v,
    E_v, S_v, Mx_v, dS_v, adot_v, amem_v, oC_v, oT_v,
    attn_v, xh2_v, rs2_v, h2_v, df_v, x2_v, dx2_v, dat_v, daT_v, aT_v, duT_v,
    doT_v, dnT_v, dC_v, dqkvT_v, dMacc, dg_v, dMb, mem_v,
    dw1_a, dw2_a, dwqkv_a, dwo_a, vec_a, db1_a, dw1_s, dw2_s, dwo_s,
    sem_in, sem_out,
):
    def cp(src, dst, sem):
        return pltpu.make_async_copy(src, dst, sem)

    in_copies = {
        "wq": cp(wq_hbm, wraw_v.at[0], sem_in.at[0]),
        "wk": cp(wk_hbm, wraw_v.at[1], sem_in.at[1]),
        "wv": cp(wv_hbm, wraw_v.at[2], sem_in.at[2]),
        "wo": cp(wo_hbm, wo_v, sem_in.at[3]),
        "go": cp(go_hbm.at[0], go_v, sem_in.at[4]),
        "w2": cp(w2_hbm, w2_v.at[0:F, :], sem_in.at[5]),
        "w1": cp(w1_hbm, w1_v.at[0:F, :], sem_in.at[6]),
    }
    for k in range(6):
        in_copies["wm%d" % k] = cp(wmod_hbm.at[:, k * D:(k + 1) * D], wmod_v.at[k],
                                   sem_in.at[7 + k])

    def x_copy(s):
        rows = pl.ds(pl.multiple_of(s * L, L), L)
        return cp(x_hbm.at[0, rows, :], x_v.at[rows, :], sem_in.at[13 + s])

    x_copy(0).start()
    for k in ("wm0", "wm1", "wq", "wk", "wv"):
        in_copies[k].start()
    x_copy(1).start()

    row128 = lax.broadcasted_iota(jnp.int32, (128, 128), 0)
    col128 = lax.broadcasted_iota(jnp.int32, (128, 128), 1)
    bias_v[...] = jnp.where(row128 <= col128, 0.0, -1e30).astype(F32)

    def head_onehot():
        return (lax.broadcasted_iota(jnp.int32, (1024, H), 0) // 32
                == lax.broadcasted_iota(jnp.int32, (1024, H), 1))

    gsig = jax.nn.sigmoid(beta_ref[...].astype(F32)[None, :])
    gcol = jnp.sum(jnp.where(head_onehot(), gsig, 0.0), axis=1, keepdims=True)
    gT_v[...] = jnp.broadcast_to(gcol, (1024, 128))

    b1f = b1_ref[...].astype(F32)[None, :]
    for t in range(FP // 128):
        w = min(128, F - 128 * t)
        blk = jnp.broadcast_to(b1f[:, 128 * t:128 * t + w], (128, w))
        if w < 128:
            blk = jnp.concatenate([blk, jnp.zeros((128, 128 - w), F32)], axis=1)
        b1c_v[128 * t:128 * t + 128, :] = blk.T

    cf = c_ref[...].astype(F32)
    silu_c = cf * jax.nn.sigmoid(cf)
    silu16 = jnp.broadcast_to(silu_c, (16, D)).astype(BF)
    scol_v[...] = jnp.broadcast_to(silu_c, (128, D)).T

    MTs[0] = jnp.zeros((NG, 128, 128), BF)
    Ms[0] = jnp.zeros((NG, 128, 128), BF)
    for r in (vec_a, dsil_v, db1_a, dg_v, dMacc):
        r[...] = jnp.zeros(r.shape, F32)
    dMb[...] = jnp.zeros(dMb.shape, BF)
    w2_v[F:FP, :] = jnp.zeros((FP - F, D), BF)
    w1_v[F:FP, :] = jnp.zeros((FP - F, D), BF)
    aT_v[:, F:FP, :] = jnp.zeros((4, FP - F, 128), BF)
    duT_v[:, F:FP, :] = jnp.zeros((4, FP - F, 128), BF)

    Macc[...] = jnp.zeros(Macc.shape, F32)
    T_v[0] = jnp.zeros((NG, 88, L), F32)

    def mod_fwd(k, c):
        mod_v[k] = _dot(silu16, wmod_v[k])[0:8]
        return c

    in_copies["wm0"].wait()
    in_copies["wm1"].wait()
    lax.fori_loop(0, 2, mod_fwd, 0)
    x_copy(0).wait()

    row24 = lax.broadcasted_iota(jnp.int32, (24, L), 0)
    row32 = lax.broadcasted_iota(jnp.int32, (32, 128), 0)
    blockmask = (row128 // 32) == (col128 // 32)
    rowvalid128 = (row128 % 32) < DH

    def modrow(k):
        return mod_v[k, 0:1, :]

    def cat4(ref, rows):
        return jnp.concatenate([ref[b, rows, :] for b in range(4)], axis=1)

    def ln1_chunk(blk, c=0):
        x = x_v[pl.ds(pl.multiple_of(blk * 128, 128), 128), :].astype(F32)
        xhat, _ = _ln_stats(x)
        h1 = xhat * (1.0 + modrow(1)) + modrow(0)
        h1T_v[blk] = h1.astype(BF).T
        return c

    def h1_rows(s, rows):
        return jnp.concatenate([h1T_v[s * 4 + b, rows, :] for b in range(4)], axis=1)

    def proj(h, p):
        t = _dot(wqkvT_v[p * D:(p + 1) * D, :], h)
        for g in range(NG):
            T_v[p, g, 0:80, :] = t[80 * g:80 * g + 80]

    def relayout(s, p):
        dst = (QT, KT, VT)[p]
        for g in range(NG):
            for hh in range(4):
                v = T_v[p, g, 20 * hh:20 * hh + 24, :]
                if p == 2:
                    fill = jnp.where(row24 < DH + 2, 1.0, 0.0)
                else:
                    fill = 0.0
                v = jnp.where(row24 < DH, v, fill)
                v = jnp.concatenate([v, jnp.zeros((8, L), F32)], axis=0).astype(BF)
                r0 = 128 * g + 32 * hh
                for b in range(4):
                    dst[s * 4 + b, r0:r0 + 32, :] = v[:, 128 * b:128 * b + 128]
            if p > 0:
                dstN = KN if p == 1 else VN
                for b in range(4):
                    dstN[s, g, 128 * b:128 * b + 128, :] = (
                        dst[s * 4 + b, 128 * g:128 * g + 128, :].T)

    def mem_update(s):
        for g in range(NG):
            vt = jnp.concatenate(
                [VT[s * 4 + b, 128 * g:128 * g + 128, :] for b in range(4)], axis=1)
            pk = jnp.concatenate(
                [jnp.where(rowvalid128,
                           _phi(KT[s * 4 + b, 128 * g:128 * g + 128, :].astype(F32)),
                           0.0).astype(BF) for b in range(4)], axis=1)
            m = jnp.where(blockmask, _dot(vt, pk, NT), 0.0) + Macc[g]
            Macc[g] = m
            MTs[s + 1, g] = m.astype(BF)
            Ms[s + 1, g] = m.T.astype(BF)

    def wT(p, c):
        for t, nm in enumerate(("wq", "wk", "wv")):
            @pl.when(p == t)
            def _():
                in_copies[nm].wait()

        wqkvT_v[pl.ds(pl.multiple_of(p * D, 128), D), :] = wraw_v[p].T
        return c

    lax.fori_loop(0, 4, ln1_chunk, 0)
    lax.fori_loop(0, 3, wT, 0)
    x_copy(2).start()
    x_copy(3).start()
    for k in ("wm2", "wm3", "wm4", "wm5", "wo", "go", "w2", "w1"):
        in_copies[k].start()

    def phase1(s, c):
        @pl.when(s < NSEG - 1)
        def _():
            x_copy(s + 1).wait()

        for b in range(4):
            hA_v[b] = h1T_v[s * 4 + b]
        proj(h1_rows(s, slice(None)), 1)
        relayout(jnp.maximum(s - 1, 0), 0)
        proj(h1_rows(s, slice(None)), 2)
        relayout(s, 1)
        proj(cat4(hA_v, slice(None)), 0)
        relayout(s, 2)
        sn = jnp.minimum(s + 1, NSEG - 1)
        for b in range(4):
            ln1_chunk(sn * 4 + b)
        mem_update(s)
        return c

    lax.fori_loop(0, NSEG, phase1, 0)

    relayout(NSEG - 1, 0)
    for nm in ("wm2", "wm3", "wm4", "wm5", "wo", "go", "w2", "w1"):
        in_copies[nm].wait()
    lax.fori_loop(2, 6, mod_fwd, 0)

    def out_copy(s):
        rows = pl.ds(pl.multiple_of(s * L, L), L)
        return cp(go_v.at[rows, :], out_hbm.at[0, rows, :], sem_out.at[s])

    def dx_copy(t):
        rows = pl.ds(pl.multiple_of(t * 256, 256), 256)
        return cp(x_v.at[rows, :], dx_hbm.at[0, rows, :], sem_out.at[4 + t])

    w_copies = {
        "dwo": cp(dwo_s, dwo_hbm, sem_out.at[14]),
        "dw1": cp(dw1_s, dw1_hbm, sem_out.at[12]),
        "dw2": cp(dw2_s, dw2_hbm, sem_out.at[13]),
    }

    def dwm_copy(k):
        cols = pl.ds(pl.multiple_of(k * D, 128), D)
        return cp(wmod_v.at[k], dwmod_hbm.at[:, cols], sem_out.at[28 + k])

    def dwqkv_copy(p, r):
        rows = pl.ds(pl.multiple_of(r * 160, 32), 160)
        dst = (dwq_hbm, dwk_hbm, dwv_hbm)[p]
        return cp(wraw_v.at[p, rows, :], dst.at[rows, :], sem_out.at[16 + 4 * p + r])

    def mod_grads(k, c):
        dmk = jnp.sum(vec_a[k], axis=0, keepdims=True)
        dm16 = jnp.broadcast_to(dmk, (16, D)).astype(BF)
        dsil_v[...] += _dot(dm16, wmod_v[k], NT)[0:8]
        scol = scol_v[...]
        for b in range(5):
            wmod_v[k, :, 128 * b:128 * b + 128] = (
                scol * dmk[:, 128 * b:128 * b + 128]).astype(BF)
        dwm_copy(k).start()
        return c

    def phase2(it, carry):
        s = NSEG - 1 - it
        last = it == NSEG - 1
        s4 = s * 4

        def acc(prev, new):
            return jnp.where(it > 0, prev, 0.0) + new

        def rows_of(r):
            return pl.ds(pl.multiple_of(s * L + r * 128, 128), 128)

        def rb(r):
            if isinstance(r, int):
                return slice(128 * r, 128 * r + 128)
            return pl.ds(pl.multiple_of(r * 128, 128), 128)

        def phi_all(ref, g):
            rg = pl.ds(pl.multiple_of(g * 128, 128), 128)
            return jnp.concatenate(
                [jnp.where(rowvalid128, _phi(ref[s4 + b, rg, :].astype(F32)), 0.0)
                 for b in range(4)], axis=1)

        def fA(g, p, st):
            j, i = PIECES[p]
            r0 = pl.multiple_of(g * 128, 128)
            if i == 0:
                q = QT[s4 + j, pl.ds(r0, 128), :].astype(F32) * (SCALE * LOG2E)
                st["w"] = _blockdiag(q.astype(BF))
            sc = _dot(KN[s, g, 128 * i:128 * i + 128, :], st["w"])
            if i == j:
                sc = sc + jnp.concatenate([bias_v[...]] * 4, axis=1)
            S_v[p] = sc
            m = jnp.max(sc.reshape(16, 8, 512), axis=0)
            if i > 0:
                m = jnp.maximum(m, st["m"])
            st["m"] = m
            if i == j:
                Mx_v[j] = jnp.broadcast_to(jnp.max(m, axis=0, keepdims=True), (8, 512))

        def fB(g, p, st):
            j, i = PIECES[p]
            m = Mx_v[j][0:1]
            if p == 0:
                mem_v[0] = _dot(MTs[s, g], phi_all(QT, g).astype(BF))
            for hh in range(4):
                r0 = pl.multiple_of(g * 128 + hh * 32, 32)
                e = jnp.exp2(S_v[p, :, 128 * hh:128 * hh + 128]
                             - m[:, 128 * hh:128 * hh + 128]).astype(BF)
                E_v[g, hh, p] = e
                o = _dot(VT[s4 + i, pl.ds(r0, 32), :], e)
                if i > 0:
                    o = o + st["o", hh]
                st["o", hh] = o
                if i == j:
                    rl = 1.0 / o[DH:DH + 1]
                    ad = o * rl
                    nh = mem_v[0, 32 * hh:32 * hh + 32, rb(j)]
                    rd = 1.0 / (nh[DH:DH + 1] + 1e-6)
                    am = nh * rd
                    gg = gT_v[pl.ds(r0, 32), :]
                    oo = ad + gg * (am - ad)
                    oC_v[j, 20 * hh:20 * hh + 20, :] = oo[0:DH]
                    adot_v[j, pl.ds(r0, 32), :] = jnp.where(row32 == DH, rl, ad)
                    amem_v[j, pl.ds(r0, 32), :] = jnp.where(row32 == DH, rd, am)
            if i == j:
                oT_v[j, pl.ds(pl.multiple_of(g * 80, 16), 80), :] = oC_v[j].astype(BF)

        st0 = {}
        for p in range(FWD_LAG):
            fA(0, p, st0)

        def fwd_group(g):
            st = {}
            for p in range(10):
                if p + FWD_LAG < 10:
                    fA(g, p + FWD_LAG, st)
                else:
                    fA(g + 1, p + FWD_LAG - 10, st)
                fB(g, p, st)

        def fwd_body(k, c):
            fwd_group(2 * k)
            fwd_group(2 * k + 1)
            return c

        lax.fori_loop(0, NG // 2 - 1, fwd_body, 0)
        fwd_group(NG - 2)

        for r in range(4):
            dfv = go_v[rows_of(r), :].astype(F32) * modrow(5)
            df_v[rb(r), :] = dfv.astype(BF)
            vec_a[6] = vec_a[6] + _colsum8(dfv)

        def daT_rows(r0, n):
            rows = pl.ds(pl.multiple_of(r0, 16), n)
            daT_v[rows, :] = _dot(w2_v[rows, :], df_v[...], NT)

        def daT_chunk(c):
            daT_rows(c * 288, 288)

        def attn_chunk(r):
            attn_v[rb(r), :] = _dot(oT_v[r], wo_v[...], TN)

        def ln2_chunk(r):
            x2 = x_v[rows_of(r), :].astype(F32) + modrow(2) * attn_v[rb(r), :]
            xh2, rs2 = _ln_stats(x2)
            x2_v[rb(r), :] = x2
            xh2_v[rb(r), :] = xh2
            rs2_v[rb(r), :] = jnp.broadcast_to(rs2, (128, 128))
            h2_v[rb(r), :] = (xh2 * (1.0 + modrow(4)) + modrow(3)).astype(BF)

        st = {}
        for p in range(10):
            if p + FWD_LAG < 10:
                fA(NG - 1, p + FWD_LAG, st)
            if p == 4:
                daT_chunk(0)
            fB(NG - 1, p, st)
        daT_chunk(1)

        def b_body(r, c):
            daT_rows((2 + r) * 288, 96)
            attn_chunk(r)
            daT_rows((2 + r) * 288 + 96, 192)
            ln2_chunk(r)
            return c

        lax.fori_loop(0, 4, b_body, 0)

        def ffn_body(c, cc):
            npc = FR // FQ
            hs = [pl.ds(pl.multiple_of(c * FR + k * FQ, 16), FQ) for k in range(npc)]
            unext = _dot(w1_v[hs[0], :], h2_v[...], NT)
            for k, h in enumerate(hs):
                u = unext
                if k + 1 < npc:
                    unext = _dot(w1_v[hs[k + 1], :], h2_v[...], NT)
                u = u + jnp.concatenate([b1c_v[h, :]] * 4, axis=1)
                u2 = u * u
                t = jnp.tanh(u * (GELU_C + (GELU_C * GELU_A) * u2))
                hp = 0.5 + 0.5 * t
                a = (u * hp).astype(BF)
                gp = hp + (0.5 * u) * (1.0 - t * t) * (GELU_C + (3.0 * GELU_C * GELU_A) * u2)
                du = daT_v[h, :] * gp
                db1_a[h, :] += (du[:, 0:128] + du[:, 128:256]) + (du[:, 256:384] + du[:, 384:512])
                dub = du.astype(BF)
                for b in range(4):
                    aT_v[b, h, :] = a[:, rb(b)]
                    duT_v[b, h, :] = dub[:, rb(b)]
                w1n = acc(dw1_a[h, :], _dot(dub, h2_v[...]))
                dw1_a[h, :] = w1n
                dw1_s[h, :] = w1n.astype(BF)
            return cc

        lax.fori_loop(0, F // FR, ffn_body, 0)

        @pl.when(last)
        def _():
            w_copies["dw1"].start()

        def ln2b_chunk(r, dh2):
            xh2 = xh2_v[rb(r), :]
            vec_a[3] = vec_a[3] + _colsum8(dh2)
            vec_a[4] = vec_a[4] + _colsum8(dh2 * xh2)
            dx2 = go_v[rows_of(r), :].astype(F32) + _ln_bwd(
                dh2 * (1.0 + modrow(4)), xh2, rs2_v[rb(r), 0:1])
            dx2_v[rb(r), :] = dx2
            vec_a[2] = vec_a[2] + _colsum8(dx2 * attn_v[rb(r), :])
            dat_v[rb(r), :] = (dx2 * modrow(2)).astype(BF)

        def out_chunk(r, f):
            f = f + b2_ref[...].astype(F32)[None, :]
            go = go_v[rows_of(r), :].astype(F32)
            vec_a[5] = vec_a[5] + _colsum8(go * f)
            go_v[rows_of(r), :] = (x2_v[rb(r), :] + modrow(5) * f).astype(BF)

        def prep(g):
            for hh in range(4):
                r0 = g * 128 + hh * 32
                rr = slice(r0, r0 + 32)
                v = jnp.where(row24 < DH, T_v[0, g, 20 * hh:20 * hh + 24, :], 0.0)
                do = jnp.concatenate([v, jnp.zeros((8, L), F32)], axis=0)
                gg = gT_v[rr, :]
                dgacc = dg_v[rr, :]
                for j in range(4):
                    d = do[:, rb(j)]
                    ad = adot_v[j, rr, :]
                    am = amem_v[j, rr, :]
                    rl = ad[DH:DH + 1]
                    rd = am[DH:DH + 1]
                    dgacc = dgacc + d * (am - ad)
                    dd = d * (1.0 - gg) * rl
                    delta = jnp.sum(dd * ad, axis=0, keepdims=True)
                    dhi = delta.astype(BF).astype(F32)
                    dlo = delta - dhi
                    dd = jnp.where(row32 == DH, -dhi, jnp.where(row32 == DH + 1, -dlo, dd))
                    doT_v[j, rr, :] = dd.astype(BF)
                    dn = d * gg * rd
                    dden = jnp.sum(dn * am, axis=0, keepdims=True)
                    dn = jnp.where(row32 == DH, -dden, dn)
                    dnT_v[j, rr, :] = dn.astype(BF)
                dg_v[rr, :] = dgacc

        def bA(g, p):
            j, i = PIECES[p]
            r0 = pl.multiple_of(g * 128, 128)
            w = _blockdiag(doT_v[j, pl.ds(r0, 128), :])
            dp = _dot(VN[s, g, 128 * i:128 * i + 128, :], w)
            for hh in range(4):
                dS_v[p, hh] = (E_v[g, hh, p].astype(F32)
                               * dp[:, 128 * hh:128 * hh + 128]).astype(BF)

        def d_body(r, c):
            h = pl.ds(pl.multiple_of(r * 432, 16), 432)
            w2n = acc(dw2_a[h, :], _dot(cat4(aT_v, h), df_v[...]))
            dw2_a[h, :] = w2n
            dw2_s[h, :] = w2n.astype(BF)
            dh2 = _dot(duT_v[r], w1_v[...], TN)
            f = _dot(aT_v[r], w2_v[...], TN)
            ln2b_chunk(r, dh2)
            out_chunk(r, f)
            return c

        lax.fori_loop(0, 4, d_body, 0)
        out_copy(s).start()
        doc = _dot(wo_v[...], dat_v[...], NT)
        for g in range(NG):
            T_v[0, g, 0:80, :] = doc[80 * g:80 * g + 80]
        for k in range(4):
            rows = slice(160 * k, 160 * k + 160)
            won = acc(dwo_a[rows, :], _dot(cat4(oT_v, rows), dat_v[...]))
            dwo_a[rows, :] = won
            dwo_s[rows, :] = won.astype(BF)
            prep(2 * k)
            prep(2 * k + 1)
        for p in range(BWD_LAG):
            bA(0, p)

        @pl.when(last)
        def _():
            w_copies["dw2"].start()
            w_copies["dwo"].start()
            lax.fori_loop(2, 6, mod_grads, 0)

        def bB(g, p, st):
            j, i = PIECES[p]
            rg = pl.ds(pl.multiple_of(g * 128, 128), 128)
            if p == 0:
                pq = phi_all(QT, g)
                dn = cat4(dnT_v, rg)
                mem_v[0] = _dot(Ms[s, g], dn) * jnp.minimum(pq, 1.0)
                st["dm"] = _dot(dn, pq.astype(BF), NT)
            if p == 3:
                pk = phi_all(KT, g)
                vt = jnp.concatenate([VT[s4 + b, rg, :] for b in range(4)], axis=1)
                mem_v[1] = _dot(dMb[1, g], vt) * jnp.minimum(pk, 1.0)
                mem_v[2] = _dot(dMb[0, g], pk.astype(BF))
                dmn = dMacc[g] + jnp.where(blockmask, st["dm"], 0.0)
                dMacc[g] = dmn
                dMb[0, g] = dmn.astype(BF)
                dMb[1, g] = dmn.T.astype(BF)
            for hh in range(4):
                r0 = pl.multiple_of(g * 128 + hh * 32, 32)
                ds = dS_v[p, hh]
                e = E_v[g, hh, p]
                do = doT_v[j, pl.ds(r0, 32), :]
                q = QT[s4 + j, pl.ds(r0, 32), :]
                dq = _dot(KT[s4 + i, pl.ds(r0, 32), :], ds)
                if i > 0:
                    dq = dq + st["dq", hh]
                st["dq", hh] = dq
                if i == j:
                    dqf = dq * SCALE + mem_v[0, 32 * hh:32 * hh + 32, rb(j)]
                    dC_v[0, j, 20 * hh:20 * hh + 20, :] = dqf[0:DH]
                a = _dot(q, ds, NT)
                b = _dot(do, e, NT)
                if i != j:
                    a = a + st["dk", hh, i]
                    b = b + st["dv", hh, i]
                st["dk", hh, i] = a
                st["dv", hh, i] = b
                if j == 3:
                    dkf = a * SCALE + mem_v[1, 32 * hh:32 * hh + 32, rb(i)]
                    dvf = b + mem_v[2, 32 * hh:32 * hh + 32, rb(i)]
                    dC_v[1, i, 20 * hh:20 * hh + 20, :] = dkf[0:DH]
                    dC_v[2, i, 20 * hh:20 * hh + 20, :] = dvf[0:DH]

            def flush(part, blk):
                r = pl.ds(pl.multiple_of(part * D + g * 80, 16), 80)
                dqkvT_v[blk, r, :] = dC_v[part, blk].astype(BF)

            if i == j:
                flush(0, j)
            if j == 3:
                flush(1, i)
                flush(2, i)

        def bwd_group(g):
            st = {}
            for p in range(10):
                if p + BWD_LAG < 10:
                    bA(g, p + BWD_LAG)
                else:
                    bA(jnp.minimum(g + 1, NG - 1), p + BWD_LAG - 10)
                bB(g, p, st)

        def bwd_body(k, c):
            bwd_group(2 * k)
            bwd_group(2 * k + 1)
            return c

        lax.fori_loop(0, NG // 2, bwd_body, 0)

        def ln1b_chunk(r, dh1):
            xh1, rs1 = _ln_stats(x_v[rows_of(r), :].astype(F32))
            vec_a[0] = vec_a[0] + _colsum8(dh1)
            vec_a[1] = vec_a[1] + _colsum8(dh1 * xh1)
            dx = dx2_v[rb(r), :] + _ln_bwd(dh1 * (1.0 + modrow(1)), xh1, rs1)
            x_v[rows_of(r), :] = dx.astype(BF)

        def dw_piece(r, ps=(0, 1, 2)):
            rows = pl.ds(pl.multiple_of(r * 160, 32), 160)
            for p in ps:
                dw = _dot(h1_rows(s, rows), cat4(dqkvT_v, slice(p * D, (p + 1) * D)), NT)
                wn = acc(dwqkv_a[p, rows, :], dw)
                dwqkv_a[p, rows, :] = wn
                wraw_v[p, rows, :] = wn.astype(BF)

        def dw_start(r):
            @pl.when(last)
            def _():
                for p in range(3):
                    dwqkv_copy(p, r).start()

        def g1_body(k, c):
            dw_piece(k, (0,))
            dha = _dot(dqkvT_v[2 * k], wqkvT_v[...], TN)
            dhb = _dot(dqkvT_v[2 * k + 1], wqkvT_v[...], TN)
            ln1b_chunk(2 * k, dha)
            dw_piece(k, (1, 2))
            ln1b_chunk(2 * k + 1, dhb)
            dx_copy(2 * s + k).start()
            dw_start(k)
            return c

        lax.fori_loop(0, 2, g1_body, 0)

        @pl.when(last)
        def _():
            lax.fori_loop(0, 2, mod_grads, 0)
            cf = c_ref[...].astype(F32)
            csig = jax.nn.sigmoid(cf)
            dc_ref[...] = (dsil_v[0:1] * (csig * (1.0 + cf * (1.0 - csig)))).astype(BF)

        def g_body(r, c):
            dw_piece(r)
            dw_start(r)
            return c

        lax.fori_loop(2, 4, g_body, 0)
        return carry

    lax.fori_loop(0, NSEG, phase2, 0)

    db2_ref[...] = jnp.sum(vec_a[6], axis=0).astype(BF)
    for t in range(FP // 128):
        w = min(128, F - 128 * t)
        row = jnp.sum(db1_a[128 * t:128 * t + 128, :].T[:, 0:w], axis=0)
        db1_ref[128 * t:128 * t + w] = row.astype(BF)
    dgrow = jnp.sum(dg_v[...], axis=1, keepdims=True)
    dgh = jnp.sum(jnp.where(head_onehot(), dgrow, 0.0), axis=0)
    gs = jax.nn.sigmoid(beta_ref[...].astype(F32))
    dbeta_ref[...] = (dgh * gs * (1.0 - gs)).astype(BF)

    for k in w_copies:
        w_copies[k].wait()
    for k in range(6):
        dwm_copy(k).wait()
    for s in range(NSEG):
        out_copy(s).wait()
        dx_copy(2 * s).wait()
        dx_copy(2 * s + 1).wait()
        for p in range(3):
            dwqkv_copy(p, s).wait()


@jax.jit
def pallas_adaLN_cond__memory_aug_infini_attn__dense_activation_gelu__prompt_kernel(
    A_x: jax.Array,
    A_wq: jax.Array,
    A_wk: jax.Array,
    A_wv: jax.Array,
    A_wo: jax.Array,
    A_beta: jax.Array,
    B_x: jax.Array,
    B_w1: jax.Array,
    B_b1: jax.Array,
    B_w2: jax.Array,
    B_b2: jax.Array,
    c: jax.Array,
    w_mod: jax.Array,
    grad_out: jax.Array,
):
    del B_x
    sd = jax.ShapeDtypeStruct
    hbm = pl.BlockSpec(memory_space=pltpu.MemorySpace.HBM)
    vm = pl.BlockSpec(memory_space=pltpu.VMEM)
    V = pltpu.VMEM
    out_shape = (
        sd((1, S_LEN, D), BF), sd((1, S_LEN, D), BF),
        sd((D, D), BF), sd((D, D), BF), sd((D, D), BF), sd((D, D), BF),
        sd((H,), BF), sd((F, D), BF), sd((F,), BF), sd((F, D), BF), sd((D,), BF),
        sd((1, D), BF), sd((D, 6 * D), BF),
    )
    out_specs = (hbm, hbm, hbm, hbm, hbm, hbm, vm, hbm, vm, hbm, vm, vm, hbm)
    in_specs = [hbm, hbm, hbm, hbm, hbm, vm, hbm, vm, hbm, vm, vm, hbm, hbm]
    scratch = [
        V((6, D, D), BF), V((3, D, D), BF), V((3 * D, D), BF), V((D, D), BF),
        V((FP, D), BF), V((FP, D), BF), V((S_LEN, D), BF), V((S_LEN, D), BF),
        V((6, 8, D), F32), V((FP, 128), F32), V((1024, 128), F32), V((128, 128), F32),
        V((D, 128), F32), V((8, D), F32),
        V((16, D, 128), BF), V((4, D, 128), BF),
        V((16, 1024, 128), BF), V((16, 1024, 128), BF), V((16, 1024, 128), BF),
        V((NSEG, NG, L, 128), BF), V((NSEG, NG, L, 128), BF),
        V((NSEG + 1, NG, 128, 128), BF), V((NSEG + 1, NG, 128, 128), BF),
        V((NG, 128, 128), F32),
        V((3, NG, 88, L), F32),
        V((NG, 4, 10, 128, 128), BF), V((10, 128, 512), F32), V((4, 8, 512), F32),
        V((10, 4, 128, 128), BF), V((4, 1024, 128), F32), V((4, 1024, 128), F32),
        V((4, 80, 128), F32), V((4, D, 128), BF),
        V((L, D), F32), V((L, D), F32), V((L, 128), F32), V((L, D), BF), V((L, D), BF),
        V((L, D), F32), V((L, D), F32), V((L, D), BF),
        V((F, L), F32), V((4, FP, 128), BF), V((4, FP, 128), BF),
        V((4, 1024, 128), BF), V((4, 1024, 128), BF), V((3, 4, 80, 128), F32),
        V((4, 3 * D, 128), BF), V((NG, 128, 128), F32), V((1024, 128), F32),
        V((2, NG, 128, 128), BF), V((3, 128, L), F32),
        V((F, D), F32), V((F, D), F32), V((3, D, D), F32), V((D, D), F32),
        V((7, 8, D), F32), V((FP, 128), F32), V((F, D), BF), V((F, D), BF), V((D, D), BF),
        pltpu.SemaphoreType.DMA((17,)), pltpu.SemaphoreType.DMA((34,)),
    ]
    res = pl.pallas_call(
        _kernel,
        out_shape=out_shape,
        in_specs=in_specs,
        out_specs=out_specs,
        scratch_shapes=scratch,
        compiler_params=pltpu.CompilerParams(vmem_limit_bytes=120 * 1024 * 1024),
    )(A_x, A_wq, A_wk, A_wv, A_wo, A_beta, B_w1.T, B_b1, B_w2, B_b2, c, w_mod, grad_out)
    (out, dx, dwq, dwk, dwv, dwo, dbeta, dw1, db1, dw2, db2, dc, dwmod) = res
    return (out, dx, dwq, dwk, dwv, dwo, dbeta, dw1.T, db1, dw2, db2, dc, dwmod)
```

```python
import math

import jax
import jax.numpy as jnp
from jax import lax
import jax.experimental.pallas as pl
import jax.experimental.pallas.tpu as pltpu

BF = jnp.bfloat16
F32 = jnp.float32

S_LEN = 2048
D = 640
H = 32
DH = 20
NSEG = 4
L = 512
F = 1728
FP = 1792
FR = 864
FQ = 144
DM = 512
NG = 8
EPS = 1e-5
SCALE = DH ** -0.5
LOG2E = math.log2(math.e)
GELU_C = math.sqrt(2.0 / math.pi)
GELU_A = 0.044715

NN = (((1,), (0,)), ((), ()))
NT = (((1,), (1,)), ((), ()))
TN = (((0,), (0,)), ((), ()))

PIECES = [(j, i) for j in range(4) for i in range(j + 1)]
A_ORDER = [0, 2, 1, 5, 3, 4, 9, 6, 7, 8]
FWD_LAG = 6
BWD_LAG = 2


def _dot(a, b, dims=NN):
    return lax.dot_general(a, b, dims, preferred_element_type=F32)


def _blockdiag(x):
    cols = []
    for hh in range(4):
        parts = []
        if hh > 0:
            parts.append(jnp.zeros((32 * hh, 128), x.dtype))
        parts.append(x[32 * hh:32 * hh + 32])
        if hh < 3:
            parts.append(jnp.zeros((96 - 32 * hh, 128), x.dtype))
        cols.append(jnp.concatenate(parts, axis=0))
    return jnp.concatenate(cols, axis=1)


def _pack_hi(x):
    lane = lax.broadcasted_iota(jnp.int32, (32, 128), 1)
    parts = []
    for hh in range(4):
        t = x[32 * hh:32 * hh + 32]
        if hh % 2 == 0:
            t = jnp.where(lane < 64, pltpu.roll(t, 64, 1), 0.0)
        else:
            t = jnp.where(lane >= 64, t, 0.0)
        parts.append(t)
    z = jnp.zeros((64, 128), F32)
    return jnp.concatenate([jnp.concatenate([parts[0], parts[1], z], axis=0),
                            jnp.concatenate([z, parts[2], parts[3]], axis=0)],
                           axis=1).astype(BF)


def _diag_dot(lhs, w, w_hi):
    lo = _dot(lhs[0:64], w)
    hi = _dot(lhs[64:128], w_hi)
    cols = []
    for hh in range(4):
        t = hi[:, 128 * (hh // 2):128 * (hh // 2) + 128]
        cols.append(pltpu.roll(t, 64, 1) if hh % 2 == 0 else t)
    return jnp.concatenate([lo, jnp.concatenate(cols, axis=1)], axis=0)


def _c24(x):
    return jnp.concatenate([x[32 * h:32 * h + 24] for h in range(4)], axis=0)


def _c24_t(m):
    return _c24(jnp.concatenate([m, jnp.zeros((32, 128), m.dtype)], axis=0).T)


def _colsum8(v):
    r, c = v.shape
    return jnp.sum(v.reshape(r // 8, 8, c), axis=0)


def _phi(t):
    return jnp.where(t > 0, t + 1.0, jnp.exp(jnp.minimum(t, 0.0)))


def _ln_stats(x):
    mu = jnp.mean(x, axis=-1, keepdims=True)
    xc = x - mu
    var = jnp.mean(xc * xc, axis=-1, keepdims=True)
    rstd = lax.rsqrt(var + EPS)
    return xc * rstd, rstd


def _ln_bwd(dxhat, xhat, rstd):
    m1 = jnp.mean(dxhat, axis=-1, keepdims=True)
    m2 = jnp.mean(dxhat * xhat, axis=-1, keepdims=True)
    return rstd * (dxhat - m1 - xhat * m2)


def _kernel(
    x_hbm, wq_hbm, wk_hbm, wv_hbm, wo_hbm, beta_hbm, w1_hbm, b1_hbm, w2_hbm, b2_hbm,
    c_hbm, wmod_hbm, go_hbm,
    out_hbm, dx_hbm, dwq_hbm, dwk_hbm, dwv_hbm, dwo_hbm, dbeta_hbm, dw1_hbm, db1_hbm,
    dw2_hbm, db2_hbm, dc_hbm, dwmod_hbm,
    wmod_v, wraw_v, wqkvT_v, wo_v, w1_v, w2_v, x_v, go_v,
    mod_v, b1c_v, gT_v, bias_v, scol_v, dsil_v,
    h1T_v, hA_v, QT, KT, VT, KN, VN, MTs, Ms, Macc, T_v,
    E_v, S_v, Mx_v, dS_v, adot_v, amem_v, oT_v,
    attn_v, xh2_v, rs2_v, h2_v, df_v, dx2_v, dat_v, daT_v, aT_v, duT_v,
    doT_v, dnT_v, dqkvT_v, dMacc, dg_v, dMb, mem_v,
    dw1_a, dw2_a, dwqkv_a, dwo_a, vec_a, db1_a, dw1_s, dw2_s, dwo_s,
    beta_ref, b1_ref, b2_ref, c_ref, dbeta_ref, db1_ref, db2_ref, dc_ref, dsr_v,
    sem_in, sem_out,
):
    def cp(src, dst, sem):
        return pltpu.make_async_copy(src, dst, sem)

    in_copies = {
        "wq": cp(wq_hbm, wraw_v.at[0], sem_in.at[0]),
        "wk": cp(wk_hbm, wraw_v.at[1], sem_in.at[1]),
        "wv": cp(wv_hbm, wraw_v.at[2], sem_in.at[2]),
        "go": cp(go_hbm.at[0], go_v, sem_in.at[3]),
    }
    late = ["wm2", "wm3", "wm4", "wm5", "go"]
    for t, (src, dst, n) in enumerate(((wo_hbm, wo_v, D), (w2_hbm, w2_v, F), (w1_hbm, w1_v, F))):
        for b in range(5):
            late.append("w%d_%d" % (t, b))
            in_copies[late[-1]] = cp(src.at[:, 128 * b:128 * b + 128], dst.at[b, 0:n, :],
                                     sem_in.at[3])
    for k in range(6):
        in_copies["wm%d" % k] = cp(wmod_hbm.at[:, k * D:(k + 1) * D], wmod_v.at[k],
                                   sem_in.at[4 if k < 2 else 5])

    def x_copy(s):
        rows = pl.ds(pl.multiple_of(s * L, L), L)
        return cp(x_hbm.at[0, rows, :], x_v.at[rows, :], sem_in.at[6 + s])

    small_in = [cp(src, dst, sem_in.at[10]) for t, (src, dst) in enumerate(
        ((beta_hbm, beta_ref), (b1_hbm, b1_ref), (b2_hbm, b2_ref), (c_hbm, c_ref)))]
    small_out = [cp(src, dst, sem_out.at[0]) for t, (src, dst) in enumerate(
        ((dc_ref, dc_hbm), (db2_ref, db2_hbm), (dbeta_ref, dbeta_hbm), (db1_ref, db1_hbm)))]
    for cpy in small_in:
        cpy.start()
    x_copy(0).start()
    for k in ("wm0", "wm1", "wq", "wk", "wv"):
        in_copies[k].start()
    x_copy(1).start()

    def zero_body(g, c):
        for r in (MTs.at[0], Ms.at[0], dMb.at[0], dMb.at[1]):
            r[g] = jnp.zeros((96, 128), BF)
        for r in (Macc, dMacc):
            r[g] = jnp.zeros((96, 128), F32)
        db1_a[pl.ds(pl.multiple_of(g * 224, 8), 224), :] = jnp.zeros((224, 128), F32)
        dg_v[pl.ds(pl.multiple_of(g * 128, 128), 128), :] = jnp.zeros((128, 128), F32)
        T_v[0, g] = jnp.zeros((88, L), F32)
        return c

    row128 = lax.broadcasted_iota(jnp.int32, (128, 128), 0)
    col128 = lax.broadcasted_iota(jnp.int32, (128, 128), 1)
    bias_v[...] = jnp.where(row128 <= col128, 0.0, -1e30).astype(F32)

    lax.fori_loop(0, NG, zero_body, 0)
    for cpy in small_in:
        cpy.wait()

    gsig = jax.nn.sigmoid(beta_ref[...].astype(F32)[None, :])
    gmat = jnp.concatenate([jnp.broadcast_to(gsig, (128, H)),
                            jnp.zeros((128, 128 - H), F32)], axis=1).T
    for h in range(H):
        gT_v[h] = jnp.broadcast_to(gmat[h:h + 1], (8, 128))

    def gate24(h):
        return jnp.concatenate([gT_v[h]] * 3, axis=0)

    b1f = b1_ref[...].astype(F32)[None, :]
    for t in range(FP // 128):
        w = min(128, F - 128 * t)
        blk = jnp.broadcast_to(b1f[:, 128 * t:128 * t + w], (128, w))
        if w < 128:
            blk = jnp.concatenate([blk, jnp.zeros((128, 128 - w), F32)], axis=1)
        b1c_v[128 * t:128 * t + 128, :] = blk.T

    cf = c_ref[...].astype(F32)
    silu_c = cf * jax.nn.sigmoid(cf)
    silu16 = jnp.broadcast_to(silu_c, (16, D)).astype(BF)
    scol_v[...] = jnp.broadcast_to(silu_c, (128, D)).T

    for r in (vec_a, dsil_v, dsr_v):
        r[...] = jnp.zeros(r.shape, F32)
    w2_v[:, F:FP, :] = jnp.zeros((5, FP - F, 128), BF)
    w1_v[:, F:FP, :] = jnp.zeros((5, FP - F, 128), BF)
    aT_v[:, F:FP, :] = jnp.zeros((4, FP - F, 128), BF)
    duT_v[:, F:FP, :] = jnp.zeros((4, FP - F, 128), BF)


    def mod_fwd(k, c):
        mod_v[k] = _dot(silu16, wmod_v[k])[0:8]
        return c

    in_copies["wm0"].wait()
    in_copies["wm1"].wait()
    x_copy(0).wait()
    lax.fori_loop(0, 2, mod_fwd, 0)

    row24 = lax.broadcasted_iota(jnp.int32, (24, L), 0)
    r24 = lax.broadcasted_iota(jnp.int32, (24, 128), 0)
    c24 = lax.broadcasted_iota(jnp.int32, (24, 128), 1)

    def blockmasked(m):
        return jnp.concatenate(
            [jnp.where(c24 // 32 == h, m[24 * h:24 * h + 24], 0.0) for h in range(4)], axis=0)

    def phi_rows(ref, blk0, rg):
        cols = []
        for b in range(4):
            t = ref[blk0 + b, rg, :].astype(F32)
            cols.append(jnp.concatenate(
                [jnp.where(r24 < DH, _phi(t[32 * h:32 * h + 24]), 0.0) for h in range(4)],
                axis=0))
        return jnp.concatenate(cols, axis=1)

    def modrow(k):
        return mod_v[k, 0:1, :]

    def cat4(ref, rows):
        return jnp.concatenate([ref[b, rows, :] for b in range(4)], axis=1)

    def cat5(ref, rows=slice(None)):
        return jnp.concatenate([ref[b, rows, :] for b in range(5)], axis=1)

    def put5(ref, rows, val):
        for b in range(5):
            ref[b, rows, :] = val[:, 128 * b:128 * b + 128].astype(BF)

    def ln1_chunk(blk, c=0):
        x = x_v[pl.ds(pl.multiple_of(blk * 128, 128), 128), :].astype(F32)
        xhat, _ = _ln_stats(x)
        h1 = xhat * (1.0 + modrow(1)) + modrow(0)
        h1T_v[blk] = h1.T.astype(BF)
        return c

    def h1_rows(s, rows):
        return jnp.concatenate([h1T_v[s * 4 + b, rows, :] for b in range(4)], axis=1)

    def proj(h, p, g0=0, g1=NG):
        t = _dot(cat5(wqkvT_v, slice(p * D + 80 * g0, p * D + 80 * g1)), h)
        for g in range(g0, g1):
            T_v[p, g, 0:80, :] = t[80 * (g - g0):80 * (g - g0) + 80]

    def relayout(s, p):
        dst = (QT, KT, VT)[p]
        fill = jnp.where(r24 < DH + 2, 1.0, 0.0) if p == 2 else 0.0
        z8 = jnp.zeros((8, 128), F32)
        for g in range(NG):
            for b in range(4):
                parts = []
                for hh in range(4):
                    v = T_v[p, g, 20 * hh:20 * hh + 24, 128 * b:128 * b + 128]
                    parts += [jnp.where(r24 < DH, v, fill), z8]
                v = jnp.concatenate(parts, axis=0)
                dst[s * 4 + b, 128 * g:128 * g + 128, :] = v.astype(BF)
                if p > 0:
                    dstN = KN if p == 1 else VN
                    dstN[s, g, 128 * b:128 * b + 128, :] = v.T.astype(BF)

    def mem_update(s):
        for g in range(NG):
            vt = jnp.concatenate(
                [VT[s * 4 + b, 128 * g:128 * g + 128, :] for b in range(4)], axis=1)
            pk = phi_rows(KT, s * 4, slice(128 * g, 128 * g + 128)).astype(BF)
            m = blockmasked(_dot(pk, vt, NT)) + Macc[g]
            Macc[g] = m
            Ms[s + 1, g] = m.astype(BF)
            MTs[s + 1, g] = _c24_t(m).astype(BF)

    def wT(p, c):
        for t, nm in enumerate(("wq", "wk", "wv")):
            @pl.when(p == t)
            def _():
                in_copies[nm].wait()

        for b in range(5):
            wqkvT_v[b, pl.ds(pl.multiple_of(p * D, 128), D), :] = (
                wraw_v[p, 128 * b:128 * b + 128, :].T)
        return c

    lax.fori_loop(0, 4, ln1_chunk, 0)
    lax.fori_loop(0, 3, wT, 0)
    x_copy(2).start()
    x_copy(3).start()
    for k in late:
        in_copies[k].start()

    def phase1(s, c):
        @pl.when(s < NSEG - 1)
        def _():
            x_copy(s + 1).wait()

        @pl.when(s == 1)
        def _():
            for nm in late[0:4]:
                in_copies[nm].wait()

        for b in range(4):
            hA_v[b] = pltpu.bitcast(h1T_v[s * 4 + b], jnp.uint32)
        proj(h1_rows(s, slice(None)), 1)
        relayout(jnp.maximum(s - 1, 0), 0)
        proj(h1_rows(s, slice(None)), 2)
        relayout(s, 1)

        def h_copy():
            return jnp.concatenate([pltpu.bitcast(hA_v[b], BF) for b in range(4)], axis=1)

        proj(h_copy(), 0, 0, 5)
        relayout(s, 2)
        sn = jnp.minimum(s + 1, NSEG - 1)
        for b in range(4):
            ln1_chunk(sn * 4 + b)
        mem_update(s)
        proj(h_copy(), 0, 5, NG)
        mod_fwd(s + 1, 0)
        return c

    lax.fori_loop(0, NSEG, phase1, 0)

    mod_fwd(5, 0)
    relayout(NSEG - 1, 0)
    for nm in late[4:]:
        in_copies[nm].wait()

    def out_copy(s):
        rows = pl.ds(pl.multiple_of(s * L, L), L)
        return cp(go_v.at[rows, :], out_hbm.at[0, rows, :], sem_out.at[0])

    def dx_copy(t):
        rows = pl.ds(pl.multiple_of(t * 256, 256), 256)
        return cp(x_v.at[rows, :], dx_hbm.at[0, rows, :], sem_out.at[0])

    w_copies = {
        "dwo": cp(dwo_s, dwo_hbm, sem_out.at[0]),
        "dw1": cp(dw1_s, dw1_hbm, sem_out.at[0]),
        "dw2": cp(dw2_s, dw2_hbm, sem_out.at[0]),
    }

    def dwm_copy(k):
        cols = pl.ds(pl.multiple_of(k * D, 128), D)
        return cp(wmod_v.at[k], dwmod_hbm.at[:, cols], sem_out.at[0])

    def dwqkv_copy(p, r):
        rows = pl.ds(pl.multiple_of(r * 160, 32), 160)
        dst = (dwq_hbm, dwk_hbm, dwv_hbm)[p]
        return cp(wraw_v.at[p, rows, :], dst.at[rows, :], sem_out.at[0])

    def mod_grads(k, c):
        dmk = jnp.sum(vec_a[k], axis=0, keepdims=True)
        dm16 = jnp.broadcast_to(dmk, (16, D)).astype(BF)
        for t in range(DM, D, 32):
            pr = wmod_v[k, t:t + 32, :].astype(F32) * dmk
            dsr_v[t - DM:t - DM + 32, :] += (
                (pr[:, 0:128] + pr[:, 128:256]) + (pr[:, 256:384] + pr[:, 384:512])
                + pr[:, 512:640])
            wmod_v[k, t:t + 32, :] = (
                jnp.concatenate([scol_v[t:t + 32, :]] * 5, axis=1) * dmk).astype(BF)
        dsil_v[:, 0:DM] += _dot(dm16, wmod_v[k, 0:DM, :], NT)[0:8]
        wmod_v[k, 0:DM, :] = (
            jnp.concatenate([scol_v[0:DM, :]] * 5, axis=1) * dmk).astype(BF)
        dwm_copy(k).start()
        return c

    def phase2(it, carry):
        s = NSEG - 1 - it
        last = it == NSEG - 1
        s4 = s * 4

        def acc(prev, new):
            return jnp.where(it > 0, prev, 0.0) + new

        def rows_of(r):
            return pl.ds(pl.multiple_of(s * L + r * 128, 128), 128)

        def rb(r):
            if isinstance(r, int):
                return slice(128 * r, 128 * r + 128)
            return pl.ds(pl.multiple_of(r * 128, 128), 128)

        def phi_all(ref, g):
            return phi_rows(ref, s4, pl.ds(pl.multiple_of(g * 128, 128), 128))

        def fA(g, t, st):
            p = A_ORDER[t]
            j, i = PIECES[p]
            r0 = pl.multiple_of(g * 128, 128)
            kn = KN[s, g, 128 * i:128 * i + 128, :]
            if i == j:
                q = QT[s4 + j, pl.ds(r0, 128), :].astype(F32) * (SCALE * LOG2E)
                st["w"] = _blockdiag(q).astype(BF)
                sc = _diag_dot(kn, st["w"], _pack_hi(q))
                sc = sc + jnp.concatenate([bias_v[...]] * 4, axis=1)
            else:
                sc = _dot(kn, st["w"])
            S_v[p] = sc
            m = jnp.max(sc.reshape(16, 8, 512), axis=0)
            if i != j:
                m = jnp.maximum(m, st["m"])
            st["m"] = m
            if i == max(j - 1, 0):
                Mx_v[j] = jnp.broadcast_to(jnp.max(m, axis=0, keepdims=True), (8, 512))

        def fB(g, p, st):
            j, i = PIECES[p]
            outs = []
            if p == 0:
                mem_v[0] = _dot(MTs[s, g, :, 0:96], phi_all(QT, g).astype(BF))
            for hh in range(4):
                r0 = pl.multiple_of(g * 128 + hh * 32, 32)
                m = jnp.concatenate([Mx_v[j, :, 128 * hh:128 * hh + 128]] * 16, axis=0)
                e = jnp.exp2(S_v[p, :, 128 * hh:128 * hh + 128] - m)
                E_v[g, hh, p, 0:64] = e[0:64].astype(BF)
                E_v[g, hh, p, 64:128] = e[64:128].astype(BF)
                o = _dot(VT[s4 + i, pl.ds(r0, 32), :], e.astype(BF))[0:24]
                if i > 0:
                    o = o + st["o", hh]
                st["o", hh] = o
                if i == j:
                    rl = 1.0 / o[DH:DH + 1]
                    ad = o * rl
                    nh = mem_v[0, 24 * hh:24 * hh + 24, rb(j)]
                    rd = 1.0 / (nh[DH:DH + 1] + 1e-6)
                    am = nh * rd
                    gg = gate24(g * 4 + hh)
                    oo = ad + gg * (am - ad)
                    outs.append(oo[0:DH])
                    adot_v[j, pl.ds(r0, 32), :] = jnp.concatenate(
                        [ad, jnp.broadcast_to(rl, (8, 128))], axis=0)
                    amem_v[j, pl.ds(r0, 32), :] = jnp.concatenate(
                        [am, jnp.broadcast_to(rd, (8, 128))], axis=0)
            if i == j:
                oT_v[j, pl.ds(pl.multiple_of(g * 80, 16), 80), :] = (
                    jnp.concatenate(outs, axis=0).astype(BF))

        st0 = {}
        for p in range(FWD_LAG):
            fA(0, p, st0)

        def fwd_group(g):
            st = {}
            for p in range(10):
                if p + FWD_LAG < 10:
                    fA(g, p + FWD_LAG, st)
                elif p < 9:
                    fA(g + 1, p + FWD_LAG - 10, st)
                fB(g, p, st)
            fA(g + 1, FWD_LAG - 1, st)

        def fwd_body(k, c):
            for t in range(3):
                fwd_group(3 * k + t)
            return c

        lax.fori_loop(0, 2, fwd_body, 0)
        fwd_group(NG - 2)

        for r in range(4):
            dfv = go_v[rows_of(r), :].astype(F32) * modrow(5)
            put5(df_v, rb(r), dfv)
            vec_a[6] = vec_a[6] + _colsum8(dfv)

        def daT_rows(r0, n):
            rows = pl.ds(pl.multiple_of(r0, 16), n)
            daT_v[rows, :] = _dot(cat5(w2_v, rows), cat5(df_v), NT)

        def daT_chunk(c):
            daT_rows(c * 288, 288)

        def ln2_chunk(r):
            x2 = x_v[rows_of(r), :].astype(F32) + modrow(2) * attn_v[rb(r), :]
            xh2, rs2 = _ln_stats(x2)
            xh2_v[rb(r), :] = xh2
            rs2_v[rb(r), :] = jnp.broadcast_to(rs2, (128, 128))
            put5(h2_v, rb(r), xh2 * (1.0 + modrow(4)) + modrow(3))

        st = {}
        for p in range(10):
            if p + FWD_LAG < 10:
                fA(NG - 1, p + FWD_LAG, st)
            if p == 4:
                daT_chunk(0)
            fB(NG - 1, p, st)
        daT_chunk(1)

        def b_body(k, c):
            r0 = (2 + 2 * k) * 288
            daT_rows(r0, 96)
            attn_v[rb(2 * k), :] = _dot(oT_v[2 * k], cat5(wo_v), TN)
            daT_rows(r0 + 96, 240)
            ln2_chunk(2 * k)
            attn_v[rb(2 * k + 1), :] = _dot(oT_v[2 * k + 1], cat5(wo_v), TN)
            daT_rows(r0 + 336, 240)
            ln2_chunk(2 * k + 1)
            return c

        lax.fori_loop(0, 2, b_body, 0)

        def ffn_body(c, cc):
            npc = FR // FQ
            hs = [pl.ds(pl.multiple_of(c * FR + k * FQ, 16), FQ) for k in range(npc)]
            unext = _dot(cat5(w1_v, hs[0]), cat5(h2_v), NT)
            for k, h in enumerate(hs):
                u = unext
                if k + 1 < npc:
                    unext = _dot(cat5(w1_v, hs[k + 1]), cat5(h2_v), NT)
                u = u + jnp.concatenate([b1c_v[h, :]] * 4, axis=1)
                u2 = u * u
                t = jnp.tanh(u * (GELU_C + (GELU_C * GELU_A) * u2))
                hp = 0.5 + 0.5 * t
                a = u * hp
                gp = hp + (0.5 * u) * (1.0 - t * t) * (GELU_C + (3.0 * GELU_C * GELU_A) * u2)
                du = daT_v[h, :] * gp
                db1_a[h, :] += (du[:, 0:128] + du[:, 128:256]) + (du[:, 256:384] + du[:, 384:512])
                for b in range(4):
                    aT_v[b, h, :] = a[:, rb(b)].astype(BF)
                    duT_v[b, h, :] = du[:, rb(b)].astype(BF)
                w1n = acc(dw1_a[h, :], _dot(du.astype(BF), cat5(h2_v)))
                dw1_a[h, :] = w1n
                dw1_s[h, :] = w1n.astype(BF)
            return cc

        lax.fori_loop(0, F // FR, ffn_body, 0)

        @pl.when(last)
        def _():
            w_copies["dw1"].start()

        def ln2b_chunk(r, dh2):
            xh2 = xh2_v[rb(r), :]
            vec_a[3] = vec_a[3] + _colsum8(dh2)
            vec_a[4] = vec_a[4] + _colsum8(dh2 * xh2)
            dx2 = go_v[rows_of(r), :].astype(F32) + _ln_bwd(
                dh2 * (1.0 + modrow(4)), xh2, rs2_v[rb(r), 0:1])
            dx2_v[rb(r), :] = dx2
            vec_a[2] = vec_a[2] + _colsum8(dx2 * attn_v[rb(r), :])
            put5(dat_v, rb(r), dx2 * modrow(2))

        def out_chunk(r, f):
            f = f + b2_ref[...].astype(F32)[None, :]
            go = go_v[rows_of(r), :].astype(F32)
            vec_a[5] = vec_a[5] + _colsum8(go * f)
            x2 = x_v[rows_of(r), :].astype(F32) + modrow(2) * attn_v[rb(r), :]
            go_v[rows_of(r), :] = (x2 + modrow(5) * f).astype(BF)

        def prep(g):
            z8 = jnp.zeros((8, 128), F32)
            for hh in range(4):
                r0 = g * 128 + hh * 32
                rr = slice(r0, r0 + 24)
                do = jnp.where(row24 < DH, T_v[0, g, 20 * hh:20 * hh + 24, :], 0.0)
                gg = gate24(g * 4 + hh)
                dgacc = dg_v[rr, :]
                for j in range(4):
                    d = do[:, rb(j)]
                    ad = adot_v[j, rr, :]
                    am = amem_v[j, rr, :]
                    rl = jnp.concatenate([adot_v[j, r0 + 24:r0 + 32, :]] * 3, axis=0)
                    rd = jnp.concatenate([amem_v[j, r0 + 24:r0 + 32, :]] * 3, axis=0)
                    dgacc = dgacc + d * (am - ad)
                    dd = d * (1.0 - gg) * rl
                    delta = jnp.sum(dd * ad, axis=0, keepdims=True)
                    dhi = delta.astype(BF).astype(F32)
                    dlo = delta - dhi
                    dd = jnp.where(r24 == DH, -dhi, jnp.where(r24 == DH + 1, -dlo, dd))
                    doT_v[j, r0:r0 + 32, :] = jnp.concatenate([dd, z8], axis=0).astype(BF)
                    dn = d * gg * rd
                    dden = jnp.sum(dn * am, axis=0, keepdims=True)
                    dn = jnp.where(r24 == DH, -dden, dn)
                    dnT_v[j, r0:r0 + 32, :] = jnp.concatenate([dn, z8], axis=0).astype(BF)
                dg_v[rr, :] = dgacc

        def bA(g, p):
            j, i = PIECES[p]
            r0 = pl.multiple_of(g * 128, 128)
            do = doT_v[j, pl.ds(r0, 128), :]
            w = _blockdiag(do)
            vn = VN[s, g, 128 * i:128 * i + 128, :]
            if i == j:
                dp = _diag_dot(vn, w, _pack_hi(do.astype(F32)))
            else:
                dp = _dot(vn, w)
            for hh in range(4):
                dS_v[p, hh] = (E_v[g, hh, p].astype(F32)
                               * dp[:, 128 * hh:128 * hh + 128]).astype(BF)

        def d_body(r, c):
            h = pl.ds(pl.multiple_of(r * 432, 16), 432)
            w2n = acc(dw2_a[h, :], _dot(cat4(aT_v, h), cat5(df_v)))
            dw2_a[h, :] = w2n
            dw2_s[h, :] = w2n.astype(BF)
            dh2 = _dot(duT_v[r], cat5(w1_v), TN)
            f = _dot(aT_v[r], cat5(w2_v), TN)
            ln2b_chunk(r, dh2)
            out_chunk(r, f)
            return c

        lax.fori_loop(0, 4, d_body, 0)
        out_copy(s).start()
        doc = _dot(cat5(wo_v), cat5(dat_v), NT)
        for g in range(NG):
            T_v[0, g, 0:80, :] = doc[80 * g:80 * g + 80]
        for k in range(4):
            rows = slice(160 * k, 160 * k + 160)
            won = acc(dwo_a[rows, :], _dot(cat4(oT_v, rows), cat5(dat_v)))
            dwo_a[rows, :] = won
            dwo_s[rows, :] = won.astype(BF)
            prep(2 * k)
            prep(2 * k + 1)
        for p in range(BWD_LAG):
            bA(0, p)

        @pl.when(last)
        def _():
            w_copies["dw2"].start()
            w_copies["dwo"].start()
            lax.fori_loop(2, 6, mod_grads, 0)

        def bB(g, p, st):
            j, i = PIECES[p]
            rg = pl.ds(pl.multiple_of(g * 128, 128), 128)
            if p == 0:
                pq = phi_all(QT, g)
                dn = cat4(dnT_v, rg)
                mem_v[0] = _dot(Ms[s, g], dn) * jnp.minimum(pq, 1.0)
                st["pq"] = pq.astype(BF)
            if p == 3:
                pk = phi_all(KT, g)
                vt = jnp.concatenate([VT[s4 + b, rg, :] for b in range(4)], axis=1)
                mem_v[1] = _dot(dMb[1, g], vt) * jnp.minimum(pk, 1.0)
                st["pk"] = pk.astype(BF)
            if p == 7:
                mem_v[2] = _dot(dMb[0, g, :, 0:96], st["pk"])
            if p == 8:
                dm = _dot(st["pq"], cat4(dnT_v, rg), NT)
                dmn = dMacc[g] + blockmasked(dm)
                dMacc[g] = dmn
                dMb[1, g] = dmn.astype(BF)
                dMb[0, g] = _c24_t(dmn).astype(BF)
            rh = [pl.ds(pl.multiple_of(g * 128 + hh * 32, 32), 32) for hh in range(4)]

            def flush(part, blk, key, scale):
                outs = []
                for hh in range(4):
                    v = st[key(hh)] if scale is None else st[key(hh)] * scale
                    v = v + mem_v[part, 24 * hh:24 * hh + 24, rb(blk)]
                    outs.append(v[0:DH])
                r = pl.ds(pl.multiple_of(part * D + g * 80, 16), 80)
                dqkvT_v[blk, r, :] = jnp.concatenate(outs, axis=0).astype(BF)

            for hh in range(4):
                a = _dot(QT[s4 + j, rh[hh], :], dS_v[p, hh], NT)[0:24]
                st["dk", hh, i] = a if i == j else a + st["dk", hh, i]
            if j == 3:
                flush(1, i, lambda hh: ("dk", hh, i), SCALE)
            for hh in range(4):
                b = _dot(doT_v[j, rh[hh], :], E_v[g, hh, p], NT)[0:24]
                st["dv", hh, i] = b if i == j else b + st["dv", hh, i]
            if p == 7:
                flush(2, 0, lambda hh: ("dv", hh, 0), None)
            if p >= 7:
                flush(2, i, lambda hh: ("dv", hh, i), None)
            for hh in range(4):
                dq = _dot(KT[s4 + i, rh[hh], :], dS_v[p, hh])[0:24]
                st["dq", hh] = dq if i == 0 else dq + st["dq", hh]
            if i == j:
                flush(0, j, lambda hh: ("dq", hh), SCALE)

        def bwd_group(g):
            st = {}
            for p in range(10):
                if p + BWD_LAG < 10:
                    bA(g, p + BWD_LAG)
                else:
                    bA(jnp.minimum(g + 1, NG - 1), p + BWD_LAG - 10)
                bB(g, p, st)

        def bwd_body(k, c):
            bwd_group(2 * k)
            bwd_group(2 * k + 1)
            return c

        lax.fori_loop(0, NG // 2, bwd_body, 0)

        def ln1b_chunk(r, dh1):
            xh1, rs1 = _ln_stats(x_v[rows_of(r), :].astype(F32))
            vec_a[0] = vec_a[0] + _colsum8(dh1)
            vec_a[1] = vec_a[1] + _colsum8(dh1 * xh1)
            dx = dx2_v[rb(r), :] + _ln_bwd(dh1 * (1.0 + modrow(1)), xh1, rs1)
            x_v[rows_of(r), :] = dx.astype(BF)

        def dw_piece(r, ps=(0, 1, 2)):
            rows = pl.ds(pl.multiple_of(r * 160, 32), 160)
            for p in ps:
                dw = _dot(h1_rows(s, rows), cat4(dqkvT_v, slice(p * D, (p + 1) * D)), NT)
                wn = acc(dwqkv_a[p, rows, :], dw)
                dwqkv_a[p, rows, :] = wn
                wraw_v[p, rows, :] = wn.astype(BF)

        def dw_start(r):
            @pl.when(last)
            def _():
                for p in range(3):
                    dwqkv_copy(p, r).start()

        def g1_body(k, c):
            dw_piece(k, (0,))
            dq2 = jnp.concatenate([dqkvT_v[2 * k], dqkvT_v[2 * k + 1]], axis=1)
            dh = _dot(dq2, cat5(wqkvT_v), TN)
            dw_piece(k, (1, 2))
            ln1b_chunk(2 * k, dh[0:128])
            ln1b_chunk(2 * k + 1, dh[128:256])
            dx_copy(2 * s + k).start()
            dw_start(k)
            return c

        lax.fori_loop(0, 2, g1_body, 0)

        @pl.when(last)
        def _():
            lax.fori_loop(0, 2, mod_grads, 0)
            db2_ref[...] = jnp.sum(vec_a[6], axis=0).astype(BF)
            small_out[1].start()

        def g_body(r, c):
            dw_piece(r)
            dw_start(r)
            return c

        lax.fori_loop(2, 4, g_body, 0)
        return carry

    lax.fori_loop(0, NSEG, phase2, 0)

    cf = c_ref[...].astype(F32)
    csig = jax.nn.sigmoid(cf)
    dsil = jnp.concatenate(
        [dsil_v[0:1, 0:DM], jnp.sum(dsr_v[...].T, axis=0, keepdims=True)], axis=1)
    dc_ref[...] = (dsil * (csig * (1.0 + cf * (1.0 - csig)))).astype(BF)
    part = db1_a[...]
    hi = part.astype(BF)
    lo = (part - hi.astype(F32)).astype(BF)
    rsum = _dot(jnp.ones((16, 256), BF), jnp.concatenate([hi, lo], axis=1), NT)
    for t in range(FP // 128):
        w = min(128, F - 128 * t)
        db1_ref[128 * t:128 * t + w] = rsum[0, 128 * t:128 * t + w].astype(BF)
    dgm = jnp.sum(dg_v[...].reshape(H, 32, 128), axis=1)
    dgm = jnp.concatenate([dgm, jnp.zeros((128 - H, 128), F32)], axis=0).T
    dgh = jnp.sum(dgm[:, 0:H], axis=0)
    gs = jax.nn.sigmoid(beta_ref[...].astype(F32))
    dbeta_ref[...] = (dgh * gs * (1.0 - gs)).astype(BF)
    small_out[0].start()
    small_out[2].start()
    small_out[3].start()

    for k in w_copies:
        w_copies[k].wait()
    for k in range(6):
        dwm_copy(k).wait()
    for s in range(NSEG):
        out_copy(s).wait()
        dx_copy(2 * s).wait()
        dx_copy(2 * s + 1).wait()
        for p in range(3):
            dwqkv_copy(p, s).wait()
    for cpy in small_out:
        cpy.wait()


@jax.jit
def pallas_adaLN_cond__memory_aug_infini_attn__dense_activation_gelu__prompt_kernel(
    A_x: jax.Array,
    A_wq: jax.Array,
    A_wk: jax.Array,
    A_wv: jax.Array,
    A_wo: jax.Array,
    A_beta: jax.Array,
    B_x: jax.Array,
    B_w1: jax.Array,
    B_b1: jax.Array,
    B_w2: jax.Array,
    B_b2: jax.Array,
    c: jax.Array,
    w_mod: jax.Array,
    grad_out: jax.Array,
):
    del B_x
    sd = jax.ShapeDtypeStruct
    hbm = pl.BlockSpec(memory_space=pltpu.MemorySpace.HBM)
    V = pltpu.VMEM
    out_shape = (
        sd((1, S_LEN, D), BF), sd((1, S_LEN, D), BF),
        sd((D, D), BF), sd((D, D), BF), sd((D, D), BF), sd((D, D), BF),
        sd((H,), BF), sd((F, D), BF), sd((F,), BF), sd((F, D), BF), sd((D,), BF),
        sd((1, D), BF), sd((D, 6 * D), BF),
    )
    out_specs = (hbm,) * 13
    in_specs = [hbm] * 13
    scratch = [
        V((6, D, D), BF), V((3, D, D), BF), V((5, 3 * D, 128), BF), V((5, D, 128), BF),
        V((5, FP, 128), BF), V((5, FP, 128), BF), V((S_LEN, D), BF), V((S_LEN, D), BF),
        V((6, 8, D), F32), V((FP, 128), F32), V((H, 8, 128), F32), V((128, 128), F32),
        V((D, 128), F32), V((8, D), F32),
        V((16, D, 128), BF), V((4, D // 2, 128), jnp.uint32),
        V((16, 1024, 128), BF), V((16, 1024, 128), BF), V((16, 1024, 128), BF),
        V((NSEG, NG, L, 128), BF), V((NSEG, NG, L, 128), BF),
        V((NSEG + 1, NG, 96, 128), BF), V((NSEG + 1, NG, 96, 128), BF),
        V((NG, 96, 128), F32),
        V((3, NG, 88, L), F32),
        V((NG, 4, 10, 128, 128), BF), V((10, 128, 512), F32), V((4, 8, 512), F32),
        V((10, 4, 128, 128), BF), V((4, 1024, 128), F32), V((4, 1024, 128), F32),
        V((4, D, 128), BF),
        V((L, D), F32), V((L, D), F32), V((L, 128), F32), V((5, L, 128), BF),
        V((5, L, 128), BF), V((L, D), F32), V((5, L, 128), BF),
        V((F, L), F32), V((4, FP, 128), BF), V((4, FP, 128), BF),
        V((4, 1024, 128), BF), V((4, 1024, 128), BF),
        V((4, 3 * D, 128), BF), V((NG, 96, 128), F32), V((1024, 128), F32),
        V((2, NG, 96, 128), BF), V((3, 96, L), F32),
        V((F, D), F32), V((F, D), F32), V((3, D, D), F32), V((D, D), F32),
        V((7, 8, D), F32), V((FP, 128), F32), V((F, D), BF), V((F, D), BF), V((D, D), BF),
        V((H,), BF), V((F,), BF), V((D,), BF), V((1, D), BF),
        V((H,), BF), V((F,), BF), V((D,), BF), V((1, D), BF),
        V((D - DM, 128), F32),
        pltpu.SemaphoreType.DMA((11,)), pltpu.SemaphoreType.DMA((1,)),
    ]
    res = pl.pallas_call(
        _kernel,
        out_shape=out_shape,
        in_specs=in_specs,
        out_specs=out_specs,
        scratch_shapes=scratch,
        compiler_params=pltpu.CompilerParams(vmem_limit_bytes=120 * 1024 * 1024),
    )(A_x, A_wq, A_wk, A_wv, A_wo, A_beta, B_w1.T, B_b1, B_w2, B_b2, c, w_mod, grad_out)
    (out, dx, dwq, dwk, dwv, dwo, dbeta, dw1, db1, dw2, db2, dc, dwmod) = res
    return (out, dx, dwq, dwk, dwv, dwo, dbeta, dw1.T, db1, dw2, db2, dc, dwmod)
```
